```python
import os as _os
_os.environ.setdefault("JAX_PLATFORMS", "cpu")
import jax
import jax.numpy as jnp

def _softmax(x, axis=-1):
    return jax.nn.softmax(x, axis=axis)
def _gelu(x):
    return jax.nn.gelu(x, approximate=True)
def _silu(x):
    return jax.nn.silu(x)
def _sigmoid(x):
    return jax.nn.sigmoid(x)
def _layernorm(x, axis=-1, eps=1e-5):
    m = jnp.mean(x, axis=axis, keepdims=True)
    v = jnp.var(x, axis=axis, keepdims=True)
    return (x - m) / jnp.sqrt(v + eps)
def _scatter_add(tgt, idx, src, axis=0):
    return tgt.at[idx].add(src)
def _segment_sum(src, seg, n):
    return jax.ops.segment_sum(src, seg, n)
class _Rng:
    def __init__(self, key):
        self._k = key
    def _next(self):
        self._k, sub = jax.random.split(self._k)
        return sub
    def normal(self, shape):
        return jax.random.normal(self._next(), shape, dtype=jnp.bfloat16)
    def randint(self, lo, hi, shape):
        return jax.random.randint(self._next(), shape, lo, hi, dtype=jnp.int32)
    def uniform(self, shape, lo=0.0, hi=1.0):
        return jax.random.uniform(self._next(), shape, jnp.bfloat16, lo, hi)
    def permutation(self, n):
        return jax.random.permutation(self._next(), n)


kernel_name = 'concat_heads__gqa_block_cached__mha_block_cached__near_ridge'

def setup_inputs():
    _rng = _Rng(jax.random.key(int.from_bytes(__import__("os").urandom(4), "little")))
    _w = (lambda a: (lambda t: t.astype(jnp.bfloat16) if jnp.issubdtype(t.dtype, jnp.floating) else t)(jnp.asarray(a)))
    def _A_setup():
        B, Sq, D = 16, 32, 1024
        Hq, Hkv, Sk, Dh = 32, 4, 32, 128
        assert Hq % Hkv == 0, (Hq, Hkv)
        return {
            "x": _w((lambda *s: _rng.normal(s) * 0.8)(B, Sq, D)),
            "k_cache": _w((lambda *s: _rng.normal(s) * 0.8)(B, Hkv, Sk, Dh)),
            "v_cache": _w((lambda *s: _rng.normal(s) * 0.05)(B, Hkv, Sk, Dh)),
            "wq": _w((lambda *s: _rng.normal(s) * 0.8)(D, Hq * Dh) * (D ** -0.5)),
            "wo": _w((lambda *s: _rng.normal(s) * 0.05)(Hq * Dh, D) * ((Hq * Dh) ** -0.5)),
        }
    _A_in = _A_setup()

    def _B_setup():
        B, Sq, D = 16, 32, 1024
        H, Sk, Dh = 32, 32, 128
        return {
            "x": _w((lambda *s: _rng.normal(s) * 0.8)(B, Sq, D)),
            "k_cache": _w((lambda *s: _rng.normal(s) * 0.8)(B, H, Sk, Dh)),
            "v_cache": _w((lambda *s: _rng.normal(s) * 0.05)(B, H, Sk, Dh)),
            "wq": _w((lambda *s: _rng.normal(s) * 0.8)(D, H * Dh) * (D ** -0.5)),
            "wo": _w((lambda *s: _rng.normal(s) * 0.05)(H * Dh, D) * ((H * Dh) ** -0.5)),
        }
    _B_in = _B_setup()

    return {
        "A_x": _A_in["x"],
        "A_k_cache": _A_in["k_cache"],
        "A_v_cache": _A_in["v_cache"],
        "A_wq": _A_in["wq"],
        "A_wo": _A_in["wo"],
        "B_x": _B_in["x"],
        "B_k_cache": _B_in["k_cache"],
        "B_v_cache": _B_in["v_cache"],
        "B_wq": _B_in["wq"],
        "B_wo": _B_in["wo"],
    }

def reference(A_x, A_k_cache, A_v_cache, A_wq, A_wo, B_x, B_k_cache, B_v_cache, B_wq, B_wo):
    def _A_ref(x, k_cache, v_cache, wq, wo):
        B, Sq, D = x.shape
        Hq, Dh = 32, 128
        Hkv = k_cache.shape[1]
        rep = Hq // Hkv
        q = (lambda x, *d: x.transpose(*d))((x @ wq).reshape(B, Sq, Hq, Dh), 0, 2, 1, 3)
        k = jnp.repeat(k_cache, rep, axis=1)
        v = jnp.repeat(v_cache, rep, axis=1)
        scores = jnp.einsum("bhqd,bhkd->bhqk", q, k) * (Dh ** -0.5)
        p = _softmax(scores, axis=-1)
        o = jnp.einsum("bhqk,bhkd->bhqd", p, v)
        return (lambda x, *d: x.transpose(*d))(o, 0, 2, 1, 3).reshape(B, Sq, Hq * Dh) @ wo

    def _B_ref(x, k_cache, v_cache, wq, wo):
        B, Sq, D = x.shape
        H, Dh = 32, 128
        q = (lambda x, *d: x.transpose(*d))((x @ wq).reshape(B, Sq, H, Dh), 0, 2, 1, 3)
        scores = jnp.einsum("bhqd,bhkd->bhqk", q, k_cache) * (Dh ** -0.5)
        p = _softmax(scores, axis=-1)
        o = jnp.einsum("bhqk,bhkd->bhqd", p, v_cache)
        return (lambda x, *d: x.transpose(*d))(o, 0, 2, 1, 3).reshape(B, Sq, H * Dh) @ wo

    a = _A_ref(A_x, A_k_cache, A_v_cache, A_wq, A_wo)
    b = _B_ref(B_x, B_k_cache, B_v_cache, B_wq, B_wo)
    return jnp.concatenate([a, b], axis=-1)
```

```python
import math, functools
import jax, jax.numpy as jnp
from jax.experimental import pallas as pl
from jax.experimental.pallas import tpu as pltpu

B, SQ, D, H, DH, SK = 16, 32, 1024, 32, 128, 32
M = B * SQ
HKV_A = 4
SC = (DH ** -0.5) * math.log2(math.e)
NT = (((1,), (1,)), ((), ()))
bf16 = jnp.bfloat16
f32 = jnp.float32

def build(cfg=None):
    cfg = cfg or {}
    QN = cfg.get('QN', 128)
    ON = cfg.get('ON', 256)
    wqa_chunks = cfg.get('wqa', [256, 256, 512, 1024, 1024, 1024])
    plan = [('xa', 'xa', 0, 0)]
    lo = 0
    wq_a = []
    for c in wqa_chunks:
        wq_a.append(('wqa%d' % lo, 'wqa', lo, lo + c)); lo += c
    assert lo == 4096
    plan += wq_a[:2]
    plan += [('ka0', 'ka', 0, 1), ('va0', 'va', 0, 1)]
    plan += wq_a[2:4]
    plan += [('ka1', 'ka', 1, 4), ('va1', 'va', 1, 4)]
    plan += wq_a[4:]
    plan += [('xb', 'xb', 0, 0)]
    nb = cfg.get('nb', 4)
    hb = H // nb
    for i in range(nb):
        plan += [('wqb%d' % i, 'wqb', i*hb*DH, (i+1)*hb*DH), ('kb%d' % i, 'kb', i*hb, (i+1)*hb), ('vb%d' % i, 'vb', i*hb, (i+1)*hb)]
    plan += [('woa', 'woa', 0, 1024), ('wob', 'wob', 0, 1024)]
    n_in = len(plan)
    n_out = 2 * (1024 // ON)

    def kernel(xa_h, ka_h, va_h, wqa_h, woa_h, xb_h, kb_h, vb_h, wqb_h, wob_h, out_h,
               xa, ka, va, wqa, woa, xb, kb, vb, wqb, wob, qa, qb, oa, ob, outs, sem_in, sem_out):
        hbm = dict(xa=xa_h, ka=ka_h, va=va_h, wqa=wqa_h, woa=woa_h, xb=xb_h, kb=kb_h, vb=vb_h, wqb=wqb_h, wob=wob_h)
        vm = dict(xa=xa, ka=ka, va=va, wqa=wqa, woa=woa, xb=xb, kb=kb, vb=vb, wqb=wqb, wob=wob)
        copies = []
        for i, (name, kind, lo, hi) in enumerate(plan):
            if kind[0] == 'x':
                src, dst = hbm[kind], vm[kind]
            elif kind[0] == 'w':
                src, dst = hbm[kind].at[:, lo:hi], vm[kind].at[:, lo:hi]
            else:
                src, dst = hbm[kind].at[:, lo:hi], vm[kind].at[:, lo:hi]
            c = pltpu.make_async_copy(src, dst, sem_in.at[i])
            c.start()
            copies.append(c)
        waited = set()
        def need(kind, idx):
            for i, (name, k, lo, hi) in enumerate(plan):
                if k == kind and (k[0] == 'x' or lo <= idx < hi):
                    if i not in waited:
                        copies[i].wait(); waited.add(i)
                    return
            raise KeyError

        lane = jax.lax.broadcasted_iota(jnp.int32, (32, 128), 1) // 32
        X = dict(a=xa, b=xb); WQ = dict(a=wqa, b=wqb); WO = dict(a=woa, b=wob)
        Q = dict(a=qa, b=qb); O = dict(a=oa, b=ob); Kc = dict(a=ka, b=kb); Vc = dict(a=va, b=vb)

        def qproj(mod, c0, w):
            need('x' + mod, 0); need('wq' + mod, c0); need('wq' + mod, c0 + w - 1)
            Q[mod][:, c0:c0+w] = jnp.dot(X[mod][...], WQ[mod][:, c0:c0+w], preferred_element_type=f32).astype(bf16)

        def softmax_T(c):
            m = jnp.max(c, axis=0, keepdims=True)
            e = jnp.exp2((c - m) * SC)
            l = jnp.sum(e, axis=0, keepdims=True)
            return e * (1.0 / l)

        def qk(mod, s, u):
            q = Q[mod]
            pts = []
            for j in range(4):
                b = 4 * u + j
                Q4 = jnp.concatenate([q[b*32:(b+1)*32, (4*s+i)*128:(4*s+i+1)*128] for i in range(4)], axis=0)
                if mod == 'a':
                    g = s // 2
                    need('ka', g)
                    c = jax.lax.dot_general(ka[b, g], Q4, NT, preferred_element_type=f32)
                else:
                    need('kb', 4*s)
                    K4 = kb[b, 4*s:4*s+4].reshape(128, 128)
                    st = jax.lax.dot_general(K4, Q4, NT, preferred_element_type=f32)
                    c = jnp.where(lane == 0, st[0:32], jnp.where(lane == 1, st[32:64], jnp.where(lane == 2, st[64:96], st[96:128])))
                pts.append(softmax_T(c))
            return jnp.concatenate(pts, axis=0).T

        def pv(mod, s, u, d):
            for i in range(4):
                di = d[32*i:32*(i+1)]
                L = jnp.concatenate([jnp.where(lane == j, di, 0.0) for j in range(4)], axis=0).astype(bf16)
                if mod == 'a':
                    need('va', s // 2)
                    W = jnp.concatenate([va[4*u+j, s // 2] for j in range(4)], axis=0)
                else:
                    need('vb', 4*s)
                    W = jnp.concatenate([vb[4*u+j, 4*s+i] for j in range(4)], axis=0)
                o = jnp.dot(L, W, preferred_element_type=f32)
                O[mod][u*128:(u+1)*128, (4*s+i)*128:(4*s+i+1)*128] = o.astype(bf16)

        out_copies = []
        def oproj(mod, n0, w):
            need('wo' + mod, 0)
            off = (0 if mod == 'a' else 1024) + n0
            outs[:, off:off+w] = jnp.dot(O[mod][...], WO[mod][:, n0:n0+w], preferred_element_type=f32).astype(bf16)
            c = pltpu.make_async_copy(outs.at[:, off:off+w], out_h.at[:, off:off+w], sem_out.at[len(out_copies)])
            c.start(); out_copies.append(c)

        for c0 in range(0, 512, QN):
            qproj('a', c0, QN)
        prev = None
        opieces = [(m, n0) for m in 'ab' for n0 in range(0, 1024, ON)]
        for t in range(16):
            mod, s = ('a', t) if t < 8 else ('b', t - 8)
            for u in range(4):
                d = qk(mod, s, u)
                if prev is not None:
                    pv(*prev)
                prev = (mod, s, u, d)
                if t < 15:
                    nm, ns = ('a', t + 1) if t + 1 < 8 else ('b', t + 1 - 8)
                    if (u * 128) % QN == 0:
                        qproj(nm, ns * 512 + u * 128, QN)
                else:
                    if u % 2 == 0 or ON <= 128:
                        oproj(*opieces.pop(0), ON)
        pv(*prev)
        for (m_, n0) in opieces:
            oproj(m_, n0, ON)
        for c in out_copies:
            c.wait()
        for i, c in enumerate(copies):
            if i not in waited:
                c.wait()

    @jax.jit
    def fn(A_x, A_k, A_v, A_wq, A_wo, B_x, B_k, B_v, B_wq, B_wo):
        out = pl.pallas_call(
            kernel,
            in_specs=[pl.BlockSpec(memory_space=pl.ANY)] * 10,
            out_specs=pl.BlockSpec(memory_space=pl.ANY),
            out_shape=jax.ShapeDtypeStruct((M, 2 * D), bf16),
            scratch_shapes=[
                pltpu.VMEM((M, D), bf16), pltpu.VMEM((B, HKV_A, SK, DH), bf16), pltpu.VMEM((B, HKV_A, SK, DH), bf16),
                pltpu.VMEM((D, H * DH), bf16), pltpu.VMEM((H * DH, D), bf16),
                pltpu.VMEM((M, D), bf16), pltpu.VMEM((B, H, SK, DH), bf16), pltpu.VMEM((B, H, SK, DH), bf16),
                pltpu.VMEM((D, H * DH), bf16), pltpu.VMEM((H * DH, D), bf16),
                pltpu.VMEM((M, H * DH), bf16), pltpu.VMEM((M, H * DH), bf16),
                pltpu.VMEM((M, H * DH), bf16), pltpu.VMEM((M, H * DH), bf16),
                pltpu.VMEM((M, 2 * D), bf16),
                pltpu.SemaphoreType.DMA((n_in,)), pltpu.SemaphoreType.DMA((n_out,)),
            ],
            compiler_params=pltpu.CompilerParams(vmem_limit_bytes=110 * 1024 * 1024),
            name='attn2',
        )(A_x.reshape(M, D), A_k, A_v, A_wq, A_wo, B_x.reshape(M, D), B_k, B_v, B_wq, B_wo)
        return out.reshape(B, SQ, 2 * D)
    return fn


_FN = build({})


@jax.jit
def pallas_concat_heads__gqa_block_cached__mha_block_cached__near_ridge_kernel(
    A_x: jax.Array,
    A_k_cache: jax.Array,
    A_v_cache: jax.Array,
    A_wq: jax.Array,
    A_wo: jax.Array,
    B_x: jax.Array,
    B_k_cache: jax.Array,
    B_v_cache: jax.Array,
    B_wq: jax.Array,
    B_wo: jax.Array,
):
    return _FN(A_x, A_k_cache, A_v_cache, A_wq, A_wo, B_x, B_k_cache, B_v_cache, B_wq, B_wo)
```

```python
import math
import jax
import jax.numpy as jnp
from jax.experimental import pallas as pl
from jax.experimental.pallas import tpu as pltpu

B, SQ, D, H, DH, SK = 16, 32, 1024, 32, 128, 32
M = B * SQ
HKV_A = 4
SC = (DH ** -0.5) * math.log2(math.e)
NT = (((1,), (1,)), ((), ()))
bf16 = jnp.bfloat16
f32 = jnp.float32


def build(cfg=None):
    cfg = cfg or {}
    PRO = cfg.get('PRO', [(1, 1, 0, 0), (2, 1, 1, 1), (3, 3, 2, 2), (5, 5, 5, 4), (8, 8, 8, 8)])
    LASTM = cfg.get('LASTM', 4)
    OBN = cfg.get('OBN', 128)
    P = cfg.get('P', 1)
    RCUT = cfg.get('RCUT', 13)
    scopes = cfg.get('scopes', False)
    npro = len(PRO)
    G_R = npro
    G_L = npro + 2
    n_in = npro + 6
    NL = 8 - P
    OAW = cfg.get('OAW', 8)
    QAW = cfg.get('QAW', 32)

    def kernel(xa_h, ka_h, va_h, wqa_h, woa_h, xb_h, kb_h, vb_h, wqb_h, wob_h, out_h,
               xa, xb, ka, va, wqa, wqb, kb, vb, woa, wob,
               qa, qb_pre, qb_cur, oa, ob_cur, acc, outs_a, outs_b, sem_in, sem_out):
        cp = pltpu.make_async_copy
        step = pl.program_id(0)

        def kv_a(g, s):
            return [cp(ka_h.at[:, g], ka.at[g], s), cp(va_h.at[:, g], va.at[g], s)]

        def grp_pro(g):
            s = sem_in.at[g]
            prev = PRO[g - 1] if g else (0, 0, 0, 0)
            out = []
            x0, x1 = max(prev) * 128, max(PRO[g]) * 128
            if x1 > x0:
                out.append(cp(xa_h.at[:, x0:x1], xa.at[:, x0:x1], s))
            for c in range(4):
                k0, k1 = prev[c] * 128, PRO[g][c] * 128
                if k1 > k0:
                    out.append(cp(wqa_h.at[k0:k1, c*512:(c+1)*512], wqa.at[c, k0:k1], s))
            if g == npro - 1:
                out += kv_a(0, s)
            return out

        def wqa_heads(h0, h1, s):
            out = []
            for q in range(h0 // 4, (h1 + 3) // 4):
                a, b = max(h0, 4*q), min(h1, 4*q + 4)
                out.append(cp(wqa_h.at[:, a*128:b*128], wqa.at[q, :, (a-4*q)*128:(b-4*q)*128], s))
            return out

        def grp_r(j):
            s = sem_in.at[G_R + j]
            if j == 0:
                return kv_a(1, s) + wqa_heads(16, 20, s) + kv_a(2, s) + wqa_heads(20, 16 + RCUT, s)
            out = kv_a(3, s) + wqa_heads(16 + RCUT, 32, s) + [cp(xb_h, xb, s)]
            out += [cp(wqb_h.at[:, i*1024:i*1024 + P*128], wqb.at[2*i, :, 0:P*128], s) for i in range(4)]
            return out

        def grp_l(i, gsrc):
            s = sem_in.at[G_L + i]
            return [cp(wqb_h.at[:, gsrc*1024 + P*128:gsrc*1024 + 512], wqb.at[2*i, :, P*128:512], s),
                    cp(wqb_h.at[:, gsrc*1024 + 512:(gsrc+1)*1024], wqb.at[2*i + 1], s),
                    cp(kb_h.at[:, 8*gsrc:8*gsrc+8], kb.at[i], s),
                    cp(vb_h.at[:, 8*gsrc:8*gsrc+8], vb.at[i], s),
                    cp(woa_h.at[:, gsrc*256:(gsrc+1)*256], woa.at[i], s),
                    cp(wob_h.at[gsrc*1024:(gsrc+1)*1024], wob.at[i], s)]

        def wait(cs, name):
            if scopes:
                with jax.named_scope(name):
                    for c in cs:
                        c.wait()
            else:
                for c in cs:
                    c.wait()

        def lane_blk():
            return jax.lax.broadcasted_iota(jnp.int32, (32, 128), 1) // 32

        def softmax_t(c):
            m = jnp.max(c, axis=0, keepdims=True)
            e = jnp.exp2((c - m) * SC)
            l = jnp.sum(e, axis=0, keepdims=True)
            return e * (1.0 / l)

        def qk(q_get, k_get, u, mha):
            lane = lane_blk()
            pts = []
            for j in range(4):
                b = 4 * u + j
                q4 = jnp.concatenate([q_get(b, i) for i in range(4)], axis=0)
                st = jax.lax.dot_general(k_get(b), q4, NT, preferred_element_type=f32)
                if mha:
                    st = jnp.where(lane == 0, st[0:32], jnp.where(lane == 1, st[32:64],
                                   jnp.where(lane == 2, st[64:96], st[96:128])))
                pts.append(softmax_t(st))
            return jnp.concatenate(pts, axis=0).T

        def pv(d, v_get, o_put, u):
            lane = lane_blk()
            for i in range(4):
                di = d[32*i:32*(i+1)]
                lhs = jnp.concatenate([jnp.where(lane == j, di, 0.0) for j in range(4)], axis=0).astype(bf16)
                w = jnp.concatenate([v_get(4*u+j, i) for j in range(4)], axis=0)
                o_put(u, i, jnp.dot(lhs, w, preferred_element_type=f32).astype(bf16))

        def mm(a, w):
            return jnp.dot(a, w, preferred_element_type=f32)

        def pipeline(groups, fillers, pend=(), pre=None):
            pend = list(pend)
            for k, f in enumerate(fillers):
                if pre is not None:
                    pre(k)
                grp = groups[k] if k < len(groups) else []
                new = []
                for t in range(max(len(pend), len(grp))):
                    if t < len(pend):
                        pend[t][0](pend[t][1])
                    if t < len(grp):
                        new.append((grp[t][1], grp[t][0]()))
                pend = new
                f()
            return pend

        def flush(pend):
            for pvf, d in pend:
                pvf(d)

        ob_pieces = []
        n0 = 0
        while n0 < D - 128:
            w = min(OBN, D - 128 - n0); ob_pieces.append((n0, w, 0, M)); n0 += w
        rm = M // LASTM
        ob_pieces += [(D - 128, 128, r*rm, (r+1)*rm) for r in range(LASTM)]

        def oa_copy(i):
            return cp(outs_a.at[i], out_h.at[:, i*256:(i+1)*256], sem_out.at[0])

        def ob_copy(n0, w, r0, r1):
            return cp(outs_b.at[r0:r1, n0:n0+w], out_h.at[r0:r1, D+n0:D+n0+w], sem_out.at[0])

        def phase_r():
            static_groups = [grp_pro(g) for g in range(npro)] + [grp_r(0), grp_r(1)]
            for g in static_groups:
                for c in g:
                    c.start()
            for i in range(4):
                for c in grp_l(i, i):
                    c.start()
            acc[...] = jnp.zeros_like(acc)

            def a_unit(s, u):
                qkf = lambda: qk(lambda b, i: qa[(4*s+i) // QAW, b*32:(b+1)*32, ((4*s+i) % QAW)*128:((4*s+i) % QAW + 1)*128],
                                 lambda b: ka[s // 2, b], u, False)

                def put(u_, i, val):
                    oa[(4*s+i) // OAW, u_*128:(u_+1)*128, ((4*s+i) % OAW)*128:((4*s+i) % OAW + 1)*128] = val
                pvf = lambda d: pv(d, lambda b, i: va[s // 2, b], put, u)
                return qkf, pvf
            un = [[a_unit(s, u) for u in range(4)] for s in range(8)]

            accv = [None] * 4

            def pro_dot(g, c):
                prev = PRO[g - 1] if g else (0, 0, 0, 0)
                k0, k1 = prev[c] * 128, PRO[g][c] * 128
                if k1 > k0:
                    part = mm(xa[:, k0:k1], wqa[c, k0:k1])
                    accv[c] = part if accv[c] is None else part + accv[c]

            def pro_last(c, half):
                k0 = PRO[npro - 2][c] * 128
                r0, r1 = half * 256, half * 256 + 256

                def f():
                    part = mm(xa[r0:r1, k0:D], wqa[c, k0:D]) + accv[c][r0:r1]
                    qa[4*c // QAW, r0:r1, (4*c % QAW)*128:(4*c % QAW)*128 + 512] = part.astype(bf16)
                return f

            for g in range(npro - 1):
                wait(static_groups[g], 'wait%02d' % g)
                for c in range(4):
                    pro_dot(g, c)
            wait(static_groups[npro - 1], 'wait%02d' % (npro - 1))
            fl = [pro_last(c, hf) for c in range(4) for hf in range(2)]
            pend = pipeline([[], [], un[0][0:2], un[0][2:4], un[1][0:1], un[1][1:2], un[1][2:3], un[1][3:4]], fl)

            def fa(h):
                def f():
                    qa[h // QAW, :, (h % QAW)*128:(h % QAW + 1)*128] = mm(xa[...], wqa[h // 4, :, (h % 4)*128:(h % 4 + 1)*128]).astype(bf16)
                return f

            def fb_p(i, p):
                def f():
                    qb_pre[i, p] = mm(xb[...], wqb[2*i, :, p*128:(p+1)*128]).astype(bf16)
                return f

            def pre(k):
                if k == 0:
                    wait(static_groups[npro], 'wait%02d' % npro)
                if k == RCUT:
                    wait(static_groups[npro + 1], 'wait%02d' % (npro + 1))
            u23 = un[2] + un[3]
            groups = [u23[0:2], u23[2:4], u23[4:6], u23[6:7], u23[7:8]] + [[x] for s in range(4, 7) for x in un[s]]
            groups += [un[7][0:2], un[7][2:4]]
            fl = [fa(h) for h in range(16, 32)] + [fb_p(i, p) for i in range(4) for p in range(P)]
            flush(pipeline(groups, fl, pend, pre))

        def phase_l(i, carry):
            wait(grp_l(i, 0), 'waitL')

            def fb(h):
                def f():
                    qb_cur[:, h*128:(h+1)*128] = mm(xb[...], wqb[2*i + (h+P)//4, :, ((h+P)%4)*128:((h+P)%4+1)*128]).astype(bf16)
                return f

            def fo(blk, r0, r1):
                def f():
                    outs_a[i, r0:r1, blk*128:(blk+1)*128] = mm(jnp.concatenate([oa[c, r0:r1, :] for c in range(H // OAW)], axis=1), woa[i, :, blk*128:(blk+1)*128]).astype(bf16)
                return f

            def b_unit(half, u):
                def q_get(b, hi):
                    h = 4 * half + hi
                    if h < P:
                        return qb_pre[i, h, b*32:(b+1)*32, :]
                    return qb_cur[b*32:(b+1)*32, (h-P)*128:(h-P+1)*128]
                qkf = lambda: qk(q_get, lambda b: kb[i, b, 4*half:4*half+4].reshape(128, 128), u, True)

                def put(u_, hi, val):
                    ob_cur[u_*128:(u_+1)*128, (half*4+hi)*128:(half*4+hi+1)*128] = val
                pvf = lambda d: pv(d, lambda b, hi: vb[i, b, 4*half+hi], put, u)
                return qkf, pvf

            units = [[b_unit(half, u)] for half in range(2) for u in range(4)]
            fillers = ([fb(h) for h in range(NL)] + [fo(0, r*128, (r+1)*128) for r in range(4)]
                       + [fo(1, 0, 128), fo(1, 128, M)])
            flush(pipeline([[]] * (5 - P) + units, fillers))
            for si in range(4):
                @pl.when(i == si)
                def _():
                    oa_copy(si).start()
            for (n0, w, r0, r1) in ob_pieces:
                t = mm(ob_cur[r0:r1, :], wob[i, :, n0:n0+w]) + acc[r0:r1, n0:n0+w]
                acc[r0:r1, n0:n0+w] = t
                outs_b[r0:r1, n0:n0+w] = t.astype(bf16)

                @pl.when(i == 3)
                def _():
                    ob_copy(n0, w, r0, r1).start()

            return carry

        @pl.when(step == 0)
        def _():
            phase_r()
            jax.lax.fori_loop(0, 4, phase_l, 0)
            wait([oa_copy(k) for k in range(4)] + [ob_copy(*p) for p in ob_pieces], 'waitout')

    def fn(A_x, A_k, A_v, A_wq, A_wo, B_x, B_k, B_v, B_wq, B_wo):
        V = pltpu.VMEM
        out = pl.pallas_call(
            kernel,
            grid=(2,),
            in_specs=[pl.BlockSpec(memory_space=pl.ANY)] * 10,
            out_specs=pl.BlockSpec(memory_space=pl.ANY),
            out_shape=jax.ShapeDtypeStruct((M, 2 * D), bf16),
            scratch_shapes=[
                V((M, D), bf16), V((M, D), bf16),
                V((HKV_A, B, SK, DH), bf16), V((HKV_A, B, SK, DH), bf16),
                V((8, D, 512), bf16),
                V((8, D, 512), bf16),
                V((4, B, 8, SK, DH), bf16), V((4, B, 8, SK, DH), bf16),
                V((4, H * DH, 256), bf16), V((4, 1024, D), bf16),
                V((H // QAW, M, QAW * DH), bf16), V((4, P, M, DH), bf16), V((M, NL * 128), bf16),
                V((H // OAW, M, OAW * DH), bf16), V((M, 1024), bf16),
                V((M, D), f32), V((4, M, 256), bf16), V((M, D), bf16),
                pltpu.SemaphoreType.DMA((n_in,)), pltpu.SemaphoreType.DMA((1,)),
            ],
            compiler_params=pltpu.CompilerParams(vmem_limit_bytes=110 * 1024 * 1024,
                                                 dimension_semantics=("arbitrary",),
                                                 disable_semaphore_checks=cfg.get('nosemchk', True)),
            name='attn2',
        )(A_x.reshape(M, D), A_k, A_v, A_wq, A_wo, B_x.reshape(M, D), B_k, B_v, B_wq, B_wo)
        return out.reshape(B, SQ, 2 * D)
    return jax.jit(fn)


_FN = build({})


@jax.jit
def pallas_concat_heads__gqa_block_cached__mha_block_cached__near_ridge_kernel(
    A_x: jax.Array,
    A_k_cache: jax.Array,
    A_v_cache: jax.Array,
    A_wq: jax.Array,
    A_wo: jax.Array,
    B_x: jax.Array,
    B_k_cache: jax.Array,
    B_v_cache: jax.Array,
    B_wq: jax.Array,
    B_wo: jax.Array,
):
    return _FN(A_x, A_k_cache, A_v_cache, A_wq, A_wo, B_x, B_k_cache, B_v_cache, B_wq, B_wo)
```

```python
import math

import jax
import jax.numpy as jnp
from jax.experimental import pallas as pl
from jax.experimental.pallas import tpu as pltpu

B, SQ, D, H, DH, SK = 16, 32, 1024, 32, 128, 32
M = B * SQ
HKV_A = 4
EXP2_SCALE = (DH ** -0.5) * math.log2(math.e)
NT_DIMS = (((1,), (1,)), ((), ()))
BF16 = jnp.bfloat16
F32 = jnp.float32

PRO = ((1, 1, 0, 0), (1, 1, 1, 1), (2, 2, 2, 2), (4, 4, 4, 3), (7, 7, 6, 6),
       (8, 8, 8, 8))
N_PRO = len(PRO)
R_CUT = 5
KV_NEED = {1: 0, 2: 5, 3: 13}
SEM_R = N_PRO
SEM_L = N_PRO + 1
N_SEM = SEM_L + 4
OB_PIECES = tuple((n0, 0, M) for n0 in range(0, D - 128, 128)) + tuple(
    (D - 128, r * 128, (r + 1) * 128) for r in range(4))


def _mm(a, w):
    return jnp.dot(a, w, preferred_element_type=F32)


def _lane_block():
    return jax.lax.broadcasted_iota(jnp.int32, (32, 128), 1) // 32


def _softmax_over_rows(s):
    m = jnp.max(s, axis=0, keepdims=True)
    e = jnp.exp2((s - m) * EXP2_SCALE)
    return e * (1.0 / jnp.sum(e, axis=0, keepdims=True))


def _qk(q_get, k_get, u, mha):
    lane = _lane_block()
    pts = []
    for j in range(4):
        b = 4 * u + j
        q4 = jnp.concatenate([q_get(b, i) for i in range(4)], axis=0)
        st = jax.lax.dot_general(k_get(b), q4, NT_DIMS, preferred_element_type=F32)
        if mha:
            st = jnp.where(lane == 0, st[0:32],
                           jnp.where(lane == 1, st[32:64],
                                     jnp.where(lane == 2, st[64:96], st[96:128])))
        pts.append(_softmax_over_rows(st))
    return jnp.concatenate(pts, axis=0).T


def _pv(p, v_get, o_put, u):
    lane = _lane_block()
    for i in range(4):
        pi = p[32 * i:32 * (i + 1)]
        lhs = jnp.concatenate(
            [jnp.where(lane == j, pi, 0.0) for j in range(4)], axis=0).astype(BF16)
        v4 = jnp.concatenate([v_get(4 * u + j, i) for j in range(4)], axis=0)
        o_put(u, i, _mm(lhs, v4).astype(BF16))


def _pipeline(groups, fillers, pend=(), pre=None):
    pend = list(pend)
    for k, filler in enumerate(fillers):
        if pre is not None:
            pre(k)
        grp = groups[k] if k < len(groups) else []
        new = []
        for t in range(max(len(pend), len(grp))):
            if t < len(pend):
                pend[t][0](pend[t][1])
            if t < len(grp):
                new.append((grp[t][1], grp[t][0]()))
        pend = new
        filler()
    return pend


def _wait_all(copies):
    for c in copies:
        c.wait()


def _kernel(xa_h, ka_h, va_h, wqa_h, woa_h, xb_h, kb_h, vb_h, wqb_h, wob_h, out_h,
            xa, xb, ka, va, wqa, wqb, kb, vb, woa, wob,
            qa, qb_pre, qb_cur, oa, ob_cur, acc, outs_a, outs_b, sem_in, sem_out):
    cp = pltpu.make_async_copy

    def kv_a(g, s):
        return [cp(ka_h.at[:, g], ka.at[g], s), cp(va_h.at[:, g], va.at[g], s)]

    def part2(f0, f1, s):
        out = []
        for g, need in KV_NEED.items():
            if f0 <= need < f1:
                out += kv_a(g, s)
        h0, h1 = 16 + min(f0, 16), 16 + min(f1, 16)
        for q in range(h0 // 4, (h1 + 3) // 4):
            a, b = max(h0, 4 * q), min(h1, 4 * q + 4)
            if b > a:
                out.append(cp(wqa_h.at[:, a * 128:b * 128],
                              wqa.at[q, :, (a - 4 * q) * 128:(b - 4 * q) * 128], s))
        if f0 <= 16 < f1:
            out.append(cp(xb_h, xb, s))
        for i in range(4):
            if f0 <= 16 + i < f1:
                out.append(cp(wqb_h.at[:, i * 1024:i * 1024 + 128],
                              wqb.at[2 * i, :, 0:128], s))
        return out

    def grp_pro(g):
        s = sem_in.at[g]
        prev = PRO[g - 1] if g else (0, 0, 0, 0)
        out = []
        x0, x1 = max(prev) * 128, max(PRO[g]) * 128
        if x1 > x0:
            out.append(cp(xa_h.at[:, x0:x1], xa.at[:, x0:x1], s))
        for c in range(4):
            k0, k1 = prev[c] * 128, PRO[g][c] * 128
            if k1 > k0:
                out.append(cp(wqa_h.at[k0:k1, c * 512:(c + 1) * 512],
                              wqa.at[c, k0:k1], s))
        if g == N_PRO - 1:
            out += kv_a(0, s) + part2(0, R_CUT, s)
        return out

    def l_dst(i):
        return [wqb.at[2 * i, :, 128:512], wqb.at[2 * i + 1], kb.at[i], vb.at[i],
                woa.at[i], wob.at[i]]

    def grp_l(i):
        src = [wqb_h.at[:, i * 1024 + 128:i * 1024 + 512],
               wqb_h.at[:, i * 1024 + 512:(i + 1) * 1024],
               kb_h.at[:, 8 * i:8 * i + 8], vb_h.at[:, 8 * i:8 * i + 8],
               woa_h.at[:, i * 256:(i + 1) * 256], wob_h.at[i * 1024:(i + 1) * 1024]]
        return [cp(s_, d_, sem_in.at[SEM_L + i]) for s_, d_ in zip(src, l_dst(i))]

    def oa_copy(i):
        return cp(outs_a.at[i], out_h.at[:, i * 256:(i + 1) * 256], sem_out.at[0])

    def ob_copy(n0, r0, r1):
        return cp(outs_b.at[r0:r1, n0:n0 + 128],
                  out_h.at[r0:r1, D + n0:D + n0 + 128], sem_out.at[0])

    @pl.when(pl.program_id(0) == 0)
    def _():
        groups_in = [grp_pro(g) for g in range(N_PRO)]
        groups_in.append(part2(R_CUT, 20, sem_in.at[SEM_R]))
        for g in groups_in + [grp_l(i) for i in range(4)]:
            for c in g:
                c.start()
        acc[...] = jnp.zeros_like(acc)

        def a_unit(s, u):
            def q_get(b, i):
                return qa[b * 32:(b + 1) * 32, (4 * s + i) * 128:(4 * s + i + 1) * 128]

            def o_put(u_, i, val):
                oa[u_ * 128:(u_ + 1) * 128, (4 * s + i) * 128:(4 * s + i + 1) * 128] = val

            return (lambda: _qk(q_get, lambda b: ka[s // 2, b], u, False),
                    lambda p: _pv(p, lambda b, i: va[s // 2, b], o_put, u))

        un = [[a_unit(s, u) for u in range(4)] for s in range(8)]
        part_q = [None] * 4

        def pro_dot(g, c):
            k0 = (PRO[g - 1][c] if g else 0) * 128
            k1 = PRO[g][c] * 128

            def f():
                if k1 > k0:
                    part = _mm(xa[:, k0:k1], wqa[c, k0:k1])
                    part_q[c] = part if part_q[c] is None else part + part_q[c]
                if k1 == D:
                    qa[:, c * 512:(c + 1) * 512] = part_q[c].astype(BF16)
            return f

        for g in range(N_PRO - 1):
            _wait_all(groups_in[g])
            for c in range(4):
                pro_dot(g, c)()
        _wait_all(groups_in[N_PRO - 1])
        pend = _pipeline([[], [], un[0][0:2], un[0][2:4] + un[1][0:1]],
                         [pro_dot(N_PRO - 1, c) for c in range(4)])

        def fa(h):
            def f():
                w = wqa[h // 4, :, (h % 4) * 128:(h % 4 + 1) * 128]
                qa[:, h * 128:(h + 1) * 128] = _mm(xa[...], w).astype(BF16)
            return f

        def fb_pre(i):
            def f():
                qb_pre[i] = _mm(xb[...], wqb[2 * i, :, 0:128]).astype(BF16)
            return f

        def pre(k):
            if k == R_CUT:
                _wait_all(groups_in[N_PRO])

        rest = un[1][1:4] + un[2] + un[3]
        groups = [rest[0:3], rest[3:5], rest[5:7], rest[7:9], rest[9:11]]
        groups += [[x] for s in range(4, 7) for x in un[s]]
        groups += [un[7][0:2], un[7][2:4]]
        fillers = [fa(h) for h in range(16, 32)] + [fb_pre(i) for i in range(4)]
        assert not _pipeline(groups, fillers, pend, pre)

    def loop_body(i, carry):
        _wait_all([cp(d_, d_, sem_in.at[SEM_L + i]) for d_ in l_dst(i)])

        def fb(h):
            def f():
                w = wqb[2 * i + h // 4, :, (h % 4) * 128:(h % 4 + 1) * 128]
                qb_cur[:, (h - 1) * 128:h * 128] = _mm(xb[...], w).astype(BF16)
            return f

        def fo(blk, r0, r1):
            def f():
                w = woa[i, :, blk * 128:(blk + 1) * 128]
                outs_a[i, r0:r1, blk * 128:(blk + 1) * 128] = (
                    _mm(oa[r0:r1, :], w).astype(BF16))
            return f

        def b_unit(half, u):
            def q_get(b, hi):
                h = 4 * half + hi
                if h == 0:
                    return qb_pre[i, b * 32:(b + 1) * 32, :]
                return qb_cur[b * 32:(b + 1) * 32, (h - 1) * 128:h * 128]

            def k_get(b):
                return kb[i, b, 4 * half:4 * half + 4].reshape(128, 128)

            def o_put(u_, hi, val):
                h = 4 * half + hi
                ob_cur[u_ * 128:(u_ + 1) * 128, h * 128:(h + 1) * 128] = val

            return (lambda: _qk(q_get, k_get, u, True),
                    lambda p: _pv(p, lambda b, hi: vb[i, b, 4 * half + hi], o_put, u))

        units = [[b_unit(half, u)] for half in range(2) for u in range(4)]
        fillers = ([fb(h) for h in range(1, 8)]
                   + [fo(0, r * 128, (r + 1) * 128) for r in range(4)]
                   + [fo(1, 0, 128), fo(1, 128, M)])
        assert not _pipeline([[]] * 4 + units, fillers)
        for k in range(4):
            @pl.when(i == k)
            def _():
                oa_copy(k).start()
        for n0, r0, r1 in OB_PIECES:
            t = _mm(ob_cur[r0:r1, :], wob[i, :, n0:n0 + 128]) + acc[r0:r1, n0:n0 + 128]
            acc[r0:r1, n0:n0 + 128] = t
            outs_b[r0:r1, n0:n0 + 128] = t.astype(BF16)

            @pl.when(i == 3)
            def _():
                ob_copy(n0, r0, r1).start()
        return carry

    @pl.when(pl.program_id(0) == 1)
    def _():
        jax.lax.fori_loop(0, 4, loop_body, 0)
        _wait_all([oa_copy(k) for k in range(4)] + [ob_copy(*p) for p in OB_PIECES])


@jax.jit
def pallas_concat_heads__gqa_block_cached__mha_block_cached__near_ridge_kernel(
    A_x: jax.Array,
    A_k_cache: jax.Array,
    A_v_cache: jax.Array,
    A_wq: jax.Array,
    A_wo: jax.Array,
    B_x: jax.Array,
    B_k_cache: jax.Array,
    B_v_cache: jax.Array,
    B_wq: jax.Array,
    B_wo: jax.Array,
):
    vmem = pltpu.VMEM
    out = pl.pallas_call(
        _kernel,
        grid=(2,),
        in_specs=[pl.BlockSpec(memory_space=pl.ANY)] * 10,
        out_specs=pl.BlockSpec(memory_space=pl.ANY),
        out_shape=jax.ShapeDtypeStruct((M, 2 * D), BF16),
        scratch_shapes=[
            vmem((M, D), BF16), vmem((M, D), BF16),
            vmem((HKV_A, B, SK, DH), BF16), vmem((HKV_A, B, SK, DH), BF16),
            vmem((8, D, 512), BF16), vmem((8, D, 512), BF16),
            vmem((4, B, 8, SK, DH), BF16), vmem((4, B, 8, SK, DH), BF16),
            vmem((4, H * DH, 256), BF16), vmem((4, 8 * DH, D), BF16),
            vmem((M, H * DH), BF16),
            vmem((4, M, DH), BF16), vmem((M, 7 * DH), BF16),
            vmem((M, H * DH), BF16), vmem((M, 8 * DH), BF16),
            vmem((M, D), F32),
            vmem((4, M, 256), BF16), vmem((M, D), BF16),
            pltpu.SemaphoreType.DMA((N_SEM,)),
            pltpu.SemaphoreType.DMA((1,)),
        ],
        compiler_params=pltpu.CompilerParams(
            dimension_semantics=("arbitrary",),
            vmem_limit_bytes=110 * 1024 * 1024,
            disable_semaphore_checks=True,
        ),
    )(A_x.reshape(M, D), A_k_cache, A_v_cache, A_wq, A_wo,
      B_x.reshape(M, D), B_k_cache, B_v_cache, B_wq, B_wo)
    return out.reshape(B, SQ, 2 * D)
```

```python
import math

import jax
import jax.numpy as jnp
from jax.experimental import pallas as pl
from jax.experimental.pallas import tpu as pltpu

B, SQ, D, H, DH, SK = 16, 32, 1024, 32, 128, 32
M = B * SQ
HKV_A = 4
EXP2_SCALE = (DH ** -0.5) * math.log2(math.e)
NT_DIMS = (((1,), (1,)), ((), ()))
BF16 = jnp.bfloat16
F32 = jnp.float32

PRO = ((1, 0, 0, 0), (1, 1, 1, 0), (2, 2, 1, 1), (3, 3, 3, 2), (5, 5, 4, 4),
       (7, 7, 7, 7), (8, 8, 8, 8))
N_PRO = len(PRO)
R_CUT = 7
UNITS_PER_FILLER = (0, 0, 1, 1,
                    2, 2, 1, 2, 1, 2, 1, 2, 1, 2, 1, 2, 1, 2, 1, 2, 1, 2, 2, 0)
UNIT_SLOT = tuple(k for k, n in enumerate(UNITS_PER_FILLER) for _ in range(n))
assert len(UNIT_SLOT) == 32
for _s in range(8):
    _done = _s if _s < 4 else 4 * _s - 9
    assert UNIT_SLOT[4 * _s] > _done + 1
KV_NEED = {g: UNIT_SLOT[8 * g] - 4 for g in (1, 2, 3)}
assert min(KV_NEED.values()) >= 0
SEM_R = N_PRO
SEM_L = N_PRO + 1
N_SEM = SEM_L + 4
OB_PIECES = tuple((n0, 0, M) for n0 in range(0, D - 128, 128)) + tuple(
    (D - 128, r * 128, (r + 1) * 128) for r in range(4))


def _mm(a, w):
    return jnp.dot(a, w, preferred_element_type=F32)


def _lane_block():
    return jax.lax.broadcasted_iota(jnp.int32, (32, 128), 1) // 32


def _softmax_over_rows(s):
    m = jnp.max(s, axis=0, keepdims=True)
    e = jnp.exp2((s - m) * EXP2_SCALE)
    return e * (1.0 / jnp.sum(e, axis=0, keepdims=True))


def _qk(q_get, k_get, u, mha):
    lane = _lane_block()
    pts = []
    for j in range(4):
        b = 4 * u + j
        q4 = jnp.concatenate([q_get(b, i) for i in range(4)], axis=0)
        st = jax.lax.dot_general(k_get(b), q4, NT_DIMS, preferred_element_type=F32)
        if mha:
            st = jnp.where(lane == 0, st[0:32],
                           jnp.where(lane == 1, st[32:64],
                                     jnp.where(lane == 2, st[64:96], st[96:128])))
        pts.append(_softmax_over_rows(st))
    return jnp.concatenate(pts, axis=0).T


def _pv(p, v_get, o_put, u):
    lane = _lane_block()
    for i in range(4):
        pi = p[32 * i:32 * (i + 1)]
        lhs = jnp.concatenate(
            [jnp.where(lane == j, pi, 0.0) for j in range(4)], axis=0).astype(BF16)
        v4 = jnp.concatenate([v_get(4 * u + j, i) for j in range(4)], axis=0)
        o_put(u, i, _mm(lhs, v4).astype(BF16))


def _pipeline(groups, fillers, pend=(), pre=None):
    pend = list(pend)
    for k, filler in enumerate(fillers):
        if pre is not None:
            pre(k)
        grp = groups[k] if k < len(groups) else []
        new = []
        for t in range(max(len(pend), len(grp))):
            if t < len(pend):
                pend[t][0](pend[t][1])
            if t < len(grp):
                new.append((grp[t][1], grp[t][0]()))
        pend = new
        filler()
    return pend


def _wait_all(copies):
    for c in copies:
        c.wait()


def _kernel(xa_h, ka_h, va_h, wqa_h, woa_h, xb_h, kb_h, vb_h, wqb_h, wob_h, out_h,
            xa, xb, ka, va, wqa, wqb, kb, vb, woa, wob,
            qa, qb_pre, qb_cur, oa, ob_cur, acc, outs_a, outs_b, sem_in, sem_out):
    cp = pltpu.make_async_copy

    def kv_a(g, s):
        return [cp(ka_h.at[:, g], ka.at[g], s), cp(va_h.at[:, g], va.at[g], s)]

    def part2(f0, f1, s):
        out = []
        for g, need in KV_NEED.items():
            if f0 <= need < f1:
                out += kv_a(g, s)
        h0, h1 = 16 + min(f0, 16), 16 + min(f1, 16)
        for q in range(h0 // 4, (h1 + 3) // 4):
            a, b = max(h0, 4 * q), min(h1, 4 * q + 4)
            if b > a:
                out.append(cp(wqa_h.at[:, a * 128:b * 128],
                              wqa.at[q, :, (a - 4 * q) * 128:(b - 4 * q) * 128], s))
        if f0 <= 16 < f1:
            out.append(cp(xb_h, xb, s))
        for i in range(4):
            if f0 <= 16 + i < f1:
                out.append(cp(wqb_h.at[:, i * 1024:i * 1024 + 128],
                              wqb.at[2 * i, :, 0:128], s))
        return out

    def grp_pro(g):
        s = sem_in.at[g]
        prev = PRO[g - 1] if g else (0, 0, 0, 0)
        out = []
        x0, x1 = max(prev) * 128, max(PRO[g]) * 128
        if x1 > x0:
            out.append(cp(xa_h.at[:, x0:x1], xa.at[:, x0:x1], s))
        for c in range(4):
            k0, k1 = prev[c] * 128, PRO[g][c] * 128
            if k1 > k0:
                out.append(cp(wqa_h.at[k0:k1, c * 512:(c + 1) * 512],
                              wqa.at[c, k0:k1], s))
        if g == N_PRO - 1:
            out += kv_a(0, s) + part2(0, R_CUT, s)
        return out

    def l_dst(i):
        return [wqb.at[2 * i, :, 128:512], wqb.at[2 * i + 1], kb.at[i], vb.at[i],
                woa.at[i], wob.at[i]]

    def grp_l(i):
        src = [wqb_h.at[:, i * 1024 + 128:i * 1024 + 512],
               wqb_h.at[:, i * 1024 + 512:(i + 1) * 1024],
               kb_h.at[:, 8 * i:8 * i + 8], vb_h.at[:, 8 * i:8 * i + 8],
               woa_h.at[:, i * 256:(i + 1) * 256], wob_h.at[i * 1024:(i + 1) * 1024]]
        return [cp(s_, d_, sem_in.at[SEM_L + i]) for s_, d_ in zip(src, l_dst(i))]

    def oa_copy(i):
        return cp(outs_a.at[i], out_h.at[:, i * 256:(i + 1) * 256], sem_out.at[0])

    def ob_copy(n0, r0, r1):
        return cp(outs_b.at[r0:r1, n0:n0 + 128],
                  out_h.at[r0:r1, D + n0:D + n0 + 128], sem_out.at[0])

    @pl.when(pl.program_id(0) == 0)
    def _():
        groups_in = [grp_pro(g) for g in range(N_PRO)]
        groups_in.append(part2(R_CUT, 20, sem_in.at[SEM_R]))
        for g in groups_in + [grp_l(i) for i in range(4)]:
            for c in g:
                c.start()
        acc[...] = jnp.zeros_like(acc)

        def a_unit(s, u):
            def q_get(b, i):
                return qa[b * 32:(b + 1) * 32, (4 * s + i) * 128:(4 * s + i + 1) * 128]

            def o_put(u_, i, val):
                oa[u_ * 128:(u_ + 1) * 128, (4 * s + i) * 128:(4 * s + i + 1) * 128] = val

            return (lambda: _qk(q_get, lambda b: ka[s // 2, b], u, False),
                    lambda p: _pv(p, lambda b, i: va[s // 2, b], o_put, u))

        units = [a_unit(s, u) for s in range(8) for u in range(4)]
        groups = [[units[n] for n in range(32) if UNIT_SLOT[n] == k] for k in range(24)]
        part_q = [None] * 4

        def pro_dot(g, c):
            k0 = (PRO[g - 1][c] if g else 0) * 128
            k1 = PRO[g][c] * 128

            def f():
                if k1 > k0:
                    part = _mm(xa[:, k0:k1], wqa[c, k0:k1])
                    part_q[c] = part if part_q[c] is None else part + part_q[c]
                if k1 == D:
                    qa[:, c * 512:(c + 1) * 512] = part_q[c].astype(BF16)
            return f

        for g in range(N_PRO - 1):
            _wait_all(groups_in[g])
            for c in range(4):
                pro_dot(g, c)()
        _wait_all(groups_in[N_PRO - 1])
        pend = _pipeline(groups[:4], [pro_dot(N_PRO - 1, c) for c in range(4)])

        def fa(h):
            def f():
                w = wqa[h // 4, :, (h % 4) * 128:(h % 4 + 1) * 128]
                qa[:, h * 128:(h + 1) * 128] = _mm(xa[...], w).astype(BF16)
            return f

        def fb_pre(i):
            def f():
                qb_pre[i] = _mm(xb[...], wqb[2 * i, :, 0:128]).astype(BF16)
            return f

        def pre(k):
            if k == R_CUT:
                _wait_all(groups_in[N_PRO])

        fillers = [fa(h) for h in range(16, 32)] + [fb_pre(i) for i in range(4)]
        pend = _pipeline(groups[4:], fillers, pend, pre)
        assert not pend

    def loop_body(i, carry):
        _wait_all([cp(d_, d_, sem_in.at[SEM_L + i]) for d_ in l_dst(i)])

        def fb(h):
            def f():
                w = wqb[2 * i + h // 4, :, (h % 4) * 128:(h % 4 + 1) * 128]
                qb_cur[:, (h - 1) * 128:h * 128] = _mm(xb[...], w).astype(BF16)
            return f

        def fo(blk, r0, r1):
            def f():
                w = woa[i, :, blk * 128:(blk + 1) * 128]
                outs_a[i, r0:r1, blk * 128:(blk + 1) * 128] = (
                    _mm(oa[r0:r1, :], w).astype(BF16))
            return f

        def b_unit(half, u):
            def q_get(b, hi):
                h = 4 * half + hi
                if h == 0:
                    return qb_pre[i, b * 32:(b + 1) * 32, :]
                return qb_cur[b * 32:(b + 1) * 32, (h - 1) * 128:h * 128]

            def k_get(b):
                return kb[i, b, 4 * half:4 * half + 4].reshape(128, 128)

            def o_put(u_, hi, val):
                h = 4 * half + hi
                ob_cur[u_ * 128:(u_ + 1) * 128, h * 128:(h + 1) * 128] = val

            return (lambda: _qk(q_get, k_get, u, True),
                    lambda p: _pv(p, lambda b, hi: vb[i, b, 4 * half + hi], o_put, u))

        units = [[b_unit(half, u)] for half in range(2) for u in range(4)]
        fillers = ([fb(h) for h in range(1, 8)]
                   + [fo(0, r * 128, (r + 1) * 128) for r in range(4)]
                   + [fo(1, 0, 128), fo(1, 128, M)])
        pend = _pipeline([[]] * 4 + units, fillers)
        assert not pend
        for k in range(4):
            @pl.when(i == k)
            def _():
                oa_copy(k).start()
        for n0, r0, r1 in OB_PIECES:
            t = _mm(ob_cur[r0:r1, :], wob[i, :, n0:n0 + 128]) + acc[r0:r1, n0:n0 + 128]
            acc[r0:r1, n0:n0 + 128] = t
            outs_b[r0:r1, n0:n0 + 128] = t.astype(BF16)

            @pl.when(i == 3)
            def _():
                ob_copy(n0, r0, r1).start()
        return carry

    @pl.when(pl.program_id(0) == 1)
    def _():
        jax.lax.fori_loop(0, 4, loop_body, 0)
        _wait_all([oa_copy(k) for k in range(4)] + [ob_copy(*p) for p in OB_PIECES])


@jax.jit
def pallas_concat_heads__gqa_block_cached__mha_block_cached__near_ridge_kernel(
    A_x: jax.Array,
    A_k_cache: jax.Array,
    A_v_cache: jax.Array,
    A_wq: jax.Array,
    A_wo: jax.Array,
    B_x: jax.Array,
    B_k_cache: jax.Array,
    B_v_cache: jax.Array,
    B_wq: jax.Array,
    B_wo: jax.Array,
):
    vmem = pltpu.VMEM
    out = pl.pallas_call(
        _kernel,
        grid=(2,),
        in_specs=[pl.BlockSpec(memory_space=pl.ANY)] * 10,
        out_specs=pl.BlockSpec(memory_space=pl.ANY),
        out_shape=jax.ShapeDtypeStruct((M, 2 * D), BF16),
        scratch_shapes=[
            vmem((M, D), BF16), vmem((M, D), BF16),
            vmem((HKV_A, B, SK, DH), BF16), vmem((HKV_A, B, SK, DH), BF16),
            vmem((8, D, 512), BF16), vmem((8, D, 512), BF16),
            vmem((4, B, 8, SK, DH), BF16), vmem((4, B, 8, SK, DH), BF16),
            vmem((4, H * DH, 256), BF16), vmem((4, 8 * DH, D), BF16),
            vmem((M, H * DH), BF16),
            vmem((4, M, DH), BF16), vmem((M, 7 * DH), BF16),
            vmem((M, H * DH), BF16), vmem((M, 8 * DH), BF16),
            vmem((M, D), F32),
            vmem((4, M, 256), BF16), vmem((M, D), BF16),
            pltpu.SemaphoreType.DMA((N_SEM,)),
            pltpu.SemaphoreType.DMA((1,)),
        ],
        compiler_params=pltpu.CompilerParams(
            dimension_semantics=("arbitrary",),
            vmem_limit_bytes=96 * 1024 * 1024,
            disable_semaphore_checks=True,
        ),
    )(A_x.reshape(M, D), A_k_cache, A_v_cache, A_wq, A_wo,
      B_x.reshape(M, D), B_k_cache, B_v_cache, B_wq, B_wo)
    return out.reshape(B, SQ, 2 * D)
```
